```python
import jax
import jax.numpy as jnp

def _softmax(x, axis=-1):
    return jax.nn.softmax(x, axis=axis)
def _gelu(x):
    return jax.nn.gelu(x, approximate=True)
def _silu(x):
    return jax.nn.silu(x)
def _sigmoid(x):
    return jax.nn.sigmoid(x)
def _layernorm(x, axis=-1, eps=1e-5):
    m = jnp.mean(x, axis=axis, keepdims=True)
    v = jnp.var(x, axis=axis, keepdims=True)
    return (x - m) / jnp.sqrt(v + eps)
def _scatter_add(tgt, idx, src, axis=0):
    return tgt.at[idx].add(src)
def _segment_sum(src, seg, n):
    return jax.ops.segment_sum(src, seg, n)
class _Rng:
    def __init__(self, key):
        self._k = key
    def _next(self):
        self._k, sub = jax.random.split(self._k)
        return sub
    def normal(self, shape):
        return jax.random.normal(self._next(), shape, dtype=jnp.bfloat16)
    def randint(self, lo, hi, shape):
        return jax.random.randint(self._next(), shape, lo, hi, dtype=jnp.int32)
    def uniform(self, shape, lo=0.0, hi=1.0):
        return jax.random.uniform(self._next(), shape, jnp.bfloat16, lo, hi)
    def permutation(self, n):
        return jax.random.permutation(self._next(), n)


kernel_name = 'standalone__gqa_block_cached__near_ridge'

def setup_inputs():
    _rng = _Rng(jax.random.key(int.from_bytes(__import__("os").urandom(4), "little")))
    _w = (lambda a: (lambda t: t.astype(jnp.bfloat16) if jnp.issubdtype(t.dtype, jnp.floating) else t)(jnp.asarray(a)))
    B, Sq, D = 16, 240, 640
    Hq, Hkv, Sk, Dh = 32, 32, 1024, 128
    assert Hq % Hkv == 0, (Hq, Hkv)
    return {
        "x": _w((lambda *s: _rng.normal(s) * 0.05)(B, Sq, D)),
        "k_cache": _w((lambda *s: _rng.normal(s) * 0.05)(B, Hkv, Sk, Dh)),
        "v_cache": _w((lambda *s: _rng.normal(s) * 0.05)(B, Hkv, Sk, Dh)),
        "wq": _w((lambda *s: _rng.normal(s) * 0.05)(D, Hq * Dh) * (D ** -0.5)),
        "wo": _w((lambda *s: _rng.normal(s) * 0.05)(Hq * Dh, D) * ((Hq * Dh) ** -0.5)),
    }

def reference(x, k_cache, v_cache, wq, wo):
    B, Sq, D = x.shape
    Hq, Dh = 32, 128
    Hkv = k_cache.shape[1]
    rep = Hq // Hkv
    q = (lambda x, *d: x.transpose(*d))((x @ wq).reshape(B, Sq, Hq, Dh), 0, 2, 1, 3)
    k = jnp.repeat(k_cache, rep, axis=1)
    v = jnp.repeat(v_cache, rep, axis=1)
    scores = jnp.einsum("bhqd,bhkd->bhqk", q, k) * (Dh ** -0.5)
    p = _softmax(scores, axis=-1)
    o = jnp.einsum("bhqk,bhkd->bhqd", p, v)
    return (lambda x, *d: x.transpose(*d))(o, 0, 2, 1, 3).reshape(B, Sq, Hq * Dh) @ wo
```

```python
import functools, json
import jax
import jax.numpy as jnp
import numpy as np
from jax import lax
import jax.experimental.pallas as pl
import jax.experimental.pallas.tpu as pltpu

CFG = json.loads('{"STR":3,"QFIRST":1}')
G = 4
U = 2 * G
STR = CFG.get('STR', 3)
NBUF = CFG.get('NBUF', 3)
FLAGS = {k: True for k in CFG.get("FL", [])}
LOG2E = 1.4426950408889634
CHS = CFG.get('CH', [64, 64, 64, 48])
CHO = CFG.get('CHO', [64, 64, 64, 48, 0])
ORDER = CFG.get('ORDER', 'pqpq')
PEEL = CFG.get('PEEL', 1)
RCP = CFG.get('RCP', 1)


ACT = {1: [(0, 0, 1), (1, 1, 1)], 2: [(1, 0, 1), (1, 1, -1)], 3: [(0, 1, 1), (1, 1, 1)], 4: [(0, 0, 1), (1, 0, 1)],
       5: [(0, 0, -1), (0, 1, 1)], 6: [(1, 1, 1)], 7: [(0, 0, 1)]}
MORD = CFG.get('MORD', [1, 7, 4, 5, 3, 2, 6])


def strassen_operands(i, A, Bm):
    f32, bf = jnp.float32, jnp.bfloat16
    add = lambda u, v: (u.astype(f32) + v.astype(f32)).astype(bf)
    sub = lambda u, v: (u.astype(f32) - v.astype(f32)).astype(bf)
    if i == 1: return add(A(0, 0), A(1, 1)), add(Bm(0, 0), Bm(1, 1))
    if i == 2: return add(A(1, 0), A(1, 1)), Bm(0, 0)
    if i == 3: return A(0, 0), sub(Bm(0, 1), Bm(1, 1))
    if i == 4: return A(1, 1), sub(Bm(1, 0), Bm(0, 0))
    if i == 5: return add(A(0, 0), A(0, 1)), Bm(1, 1)
    if i == 6: return sub(A(1, 0), A(0, 0)), add(Bm(0, 0), Bm(0, 1))
    if i == 7: return sub(A(0, 1), A(1, 1)), add(Bm(1, 0), Bm(1, 1))


def kernel(x_hbm, k_hbm, v_hbm, wq_hbm, wo_hbm, o_hbm,
           x_buf, wq_buf, wo_buf, kv_buf, q_buf, a_buf, acc, stage, o_acc, q_acc,
           x_sem, w_sem, kv_sem, o_sem, *bufs, B, H, Sq, Sk, D, Dh):
    s_bufs = bufs[:2]
    p_bufs = bufs[2:2 + U]
    l_bufs = bufs[2 + U:2 + 2 * U]
    NG = H // G
    NS = NG * B
    W = G * Dh
    HK = Sk // 2
    T = 256
    LB = B.bit_length() - 1
    assert B == 1 << LB
    qscale = (Dh ** -0.5) * LOG2E
    f32 = jnp.float32
    rows = lambda i: slice(i * Sq, (i + 1) * Sq)
    cols = lambda i: slice(i * T, (i + 1) * T)
    last = {(r, c): max(MORD.index(i) for i in ACT if any((r, c) == a[:2] for a in ACT[i])) for r in range(2) for c in range(2)}
    first = {(r, c): min(MORD.index(i) for i in ACT if any((r, c) == a[:2] for a in ACT[i])) for r in range(2) for c in range(2)}

    def bg(s):
        return s & (B - 1), s >> LB

    def x_copy(b):
        return pltpu.make_async_copy(x_hbm.at[b], x_buf.at[b], x_sem.at[b])

    def wq_copy(g):
        return pltpu.make_async_copy(wq_hbm.at[:, pl.ds(pl.multiple_of(g * W, W), W)], wq_buf.at[g], w_sem.at[0])

    def wo_copy(g):
        return pltpu.make_async_copy(wo_hbm.at[pl.ds(pl.multiple_of(g * W, W), W), :], wo_buf.at[g], w_sem.at[1])

    def k_copy(s, slot):
        b, g = bg(s)
        return pltpu.make_async_copy(k_hbm.at[pl.ds(2 * b, 2), pl.ds(g * G, G)], kv_buf.at[slot, 0], kv_sem.at[slot])

    def v_copy(s, slot):
        b, g = bg(s)
        return pltpu.make_async_copy(v_hbm.at[pl.ds(2 * b, 2), pl.ds(g * G, G)], kv_buf.at[slot, 1], kv_sem.at[slot])

    def kv_wait(slot):
        pltpu.make_async_copy(kv_buf.at[slot], kv_buf.at[slot], kv_sem.at[slot]).wait()

    def o_copy(b):
        return pltpu.make_async_copy(stage.at[b], o_hbm.at[b], o_sem.at[b])

    def qproj(b, g, between):
        if not STR & 1:
            for r in range(2):
                q = jnp.dot(x_buf[b, rows(r)], wq_buf[g], preferred_element_type=f32)
                q_buf[rows(r)] = (q * qscale).astype(jnp.bfloat16)
            return
        for r in range(2):
            q_acc[rows(r)] = jnp.dot(x_buf[b, rows(r), 2 * T:], wq_buf[g, 2 * T:, :], preferred_element_type=f32)
            between(r)
        for n, i in enumerate(MORD):
            lhs, rhs = strassen_operands(i, lambda r, c: x_buf[b, rows(r), cols(c)], lambda r, c: wq_buf[g, cols(r), cols(c)])
            m = jnp.dot(lhs, rhs, preferred_element_type=f32)
            for r, c, sg in ACT[i]:
                t = q_acc[rows(r), cols(c)] + m if sg > 0 else q_acc[rows(r), cols(c)] - m
                if last[r, c] == n:
                    q_buf[rows(r), cols(c)] = (t * qscale).astype(jnp.bfloat16)
                else:
                    q_acc[rows(r), cols(c)] = t
            between(2 + n)

    def oproj(b, g, between):
        def upd(r, c, m, sg, is_first, is_last):
            old = acc[b, rows(r), c]
            if is_first:
                old = jnp.where(g == 0, 0.0, old)
            t = old + m if sg > 0 else old - m
            acc[b, rows(r), c] = t
            if is_last:
                stage[b, rows(r), c] = t.astype(stage.dtype)
        if not STR & 2:
            for r in range(2):
                for n in range(5):
                    c = slice(n * 128, n * 128 + 128)
                    upd(r, c, jnp.dot(a_buf[rows(r)], wo_buf[g, :, c], preferred_element_type=f32), 1, True, True)
                    if r == 0: between(n)
            return
        for r in range(2):
            c = slice(2 * T, D)
            upd(r, c, jnp.dot(a_buf[rows(r)], wo_buf[g, :, c], preferred_element_type=f32), 1, True, True)
            between(r)
        for n, i in enumerate(MORD):
            lhs, rhs = strassen_operands(i, lambda r, c: a_buf[rows(r), cols(c)], lambda r, c: wo_buf[g, cols(r), cols(c)])
            m = jnp.dot(lhs, rhs, preferred_element_type=f32)
            for r, c, sg in ACT[i]:
                upd(r, cols(c), m, sg, first[r, c] == n, last[r, c] == n)
            between(2 + n)

    def qk(slot, u, j):
        c = slice(j * HK, (j + 1) * HK)
        r, h = divmod(u, G)
        s_bufs[u % 2][:, c] = lax.dot_general(q_buf[rows(r), h * Dh:(h + 1) * Dh], kv_buf[slot, 0, r, h, c, :],
                                              (((1,), (1,)), ((), ())), preferred_element_type=f32)

    def sm(u, chs, i):
        if i >= len(chs) or chs[i] == 0:
            return
        r0 = sum(chs[:i])
        n = chs[i]
        r = slice(r0, r0 + n)
        s = s_bufs[u % 2][r, :]
        m = jnp.max(s, axis=-1, keepdims=True)
        p = jnp.exp2(s - m)
        l = jnp.sum(p, axis=-1, keepdims=True)
        p_bufs[u][r, :] = p.astype(jnp.bfloat16)
        if RCP:
            rl = pl.reciprocal(l, approx=True)
            rl = rl * (2.0 - l * rl)
        else:
            rl = 1.0 / l
        l_bufs[u][r, :] = jnp.broadcast_to(rl, (n, Dh))

    def pv(slot, u, j):
        c = slice(j * HK, (j + 1) * HK)
        r, h = divmod(u, G)
        o = jnp.dot(p_bufs[u][:, c], kv_buf[slot, 1, r, h, c, :], preferred_element_type=f32)
        if j == 0:
            o_acc[...] = o
        else:
            a_buf[rows(r), h * Dh:(h + 1) * Dh] = ((o_acc[...] + o) * l_bufs[u][...]).astype(jnp.bfloat16)

    def compute(s, slot, front, back, mid):
        bn, gn = bg(jnp.minimum(s + 1, NS - 1))
        bp, gp = bg(jnp.maximum(s - 1, 0))
        for u in range(U):
            cnt = {'p': 0, 'q': 0}
            for i, t in enumerate(ORDER):
                if t == 'p' and back:
                    pv(slot, u, cnt[t])
                if t == 'q' and front:
                    qk(slot, u, cnt[t])
                cnt[t] += 1
                if front and u > 0:
                    sm(u - 1, CHS, i)
        mid()
        nop = lambda n: None
        smo = lambda n: sm(U - 1, CHO, n)
        if front and back:
            if CFG.get('QFIRST', 0):
                qproj(bn, gn, smo)
                oproj(bp, gp, nop)
            else:
                oproj(bp, gp, smo)
                qproj(bn, gn, nop)
        elif front:
            qproj(bn, gn, smo)
        else:
            oproj(bp, gp, nop)

    def starts(s, slot):
        b, g = bg(s)

        @pl.when(s + NBUF <= NS)
        def _():
            k_copy(jnp.minimum(s + NBUF, NS - 1), slot).start()
            v_copy(s + NBUF - 1, slot).start()

        @pl.when(s + 3 < B)
        def _():
            x_copy(s + 3).start()

        @pl.when((b == 2) & (g + 1 < NG))
        def _():
            wq_copy(g + 1).start()
            wo_copy(g + 1).start()

        @pl.when(s - 2 >= NS - B)
        def _():
            o_copy(s - 2 - (NS - B)).start()

    def waits(s, nslot):
        b, g = bg(s)

        @pl.when(s + 2 < B)
        def _():
            x_copy(s + 2).wait()

        @pl.when((b == B - 2) & (g + 1 < NG))
        def _():
            wq_copy(g + 1).wait()
            wo_copy(g + 1).wait()

        kv_wait(nslot)

    x_copy(0).start()
    wq_copy(0).start()
    k_copy(0, 0).start()
    x_copy(0).wait()
    wq_copy(0).wait()
    x_copy(1).start()
    x_copy(2).start()
    k_copy(1, 1).start()
    v_copy(0, 1).start()
    wo_copy(0).start()
    qproj(0, 0, lambda n: None)
    k_copy(0, 0).wait()
    for s in range(2, NBUF):
        k_copy(s, s).start()
        v_copy(s - 1, s).start()
    x_copy(1).wait()
    compute(0, 0, True, False, lambda: starts(0, 0))
    wo_copy(0).wait()
    waits(0, 1)

    def step(s, slot):
        nslot = jnp.where(slot == NBUF - 1, 0, slot + 1)
        compute(s, slot, True, True, lambda: starts(s, slot))
        waits(s, nslot)
        return nslot

    lax.fori_loop(1, NS, step, jnp.int32(1))
    o_copy(B - 2).start()
    compute(NS, NS % NBUF, False, True, lambda: None)
    o_copy(B - 1).start()
    for bb in range(B):
        o_copy(bb).wait()


@jax.jit
def pallas_standalone__gqa_block_cached__near_ridge_kernel(x, k_cache, v_cache, wq, wo):
    B, Sq, D = x.shape
    B //= 2
    x = x.reshape(B, 2 * Sq, D)
    _, H, Sk, Dh = k_cache.shape
    NG = H // G
    bf = jnp.bfloat16
    f32 = jnp.float32
    any_spec = pl.BlockSpec(memory_space=pl.ANY)
    return pl.pallas_call(
        functools.partial(kernel, B=B, H=H, Sq=Sq, Sk=Sk, D=D, Dh=Dh),
        in_specs=[any_spec] * 5,
        out_specs=any_spec,
        out_shape=jax.ShapeDtypeStruct((B, 2 * Sq, D), x.dtype),
        scratch_shapes=[
            pltpu.VMEM((B, 2 * Sq, D), bf),
            pltpu.VMEM((NG, D, G * Dh), bf),
            pltpu.VMEM((NG, G * Dh, D), bf),
            pltpu.VMEM((NBUF, 2, 2, G, Sk, Dh), bf),
            pltpu.VMEM((2 * Sq, G * Dh), bf),
            pltpu.VMEM((2 * Sq, G * Dh), bf),
            pltpu.VMEM((B, 2 * Sq, D), f32),
            pltpu.VMEM((B, 2 * Sq, D), x.dtype),
            pltpu.VMEM((Sq, Dh), f32),
            pltpu.VMEM((2 * Sq, G * Dh), f32),
            pltpu.SemaphoreType.DMA((B,)),
            pltpu.SemaphoreType.DMA((2,)),
            pltpu.SemaphoreType.DMA((NBUF,)),
            pltpu.SemaphoreType.DMA((B,)),
        ] + [pltpu.VMEM((Sq, Sk), f32)] * 2 + [pltpu.VMEM((Sq, Sk), bf)] * U + [pltpu.VMEM((Sq, Dh), f32)] * U,
        compiler_params=pltpu.CompilerParams(vmem_limit_bytes=100 * 1024 * 1024, disable_bounds_checks=True, flags=FLAGS),
    )(x, k_cache, v_cache, wq, wo).reshape(2 * B, Sq, D)
```

```python
import functools

import jax
import jax.numpy as jnp
from jax import lax
import jax.experimental.pallas as pl
import jax.experimental.pallas.tpu as pltpu

G = 4
U = 2 * G
T = 256
LOG2E = 1.4426950408889634
SM_ROWS = (96, 16, 32, 96)
SM_ROWS_LAST = (48, 32, 80, 80)
UPDATES = {
    1: ((0, 0, 1), (1, 1, 1)),
    2: ((1, 0, 1), (1, 1, -1)),
    3: ((0, 1, 1), (1, 1, 1)),
    4: ((0, 0, 1), (1, 0, 1)),
    5: ((0, 0, -1), (0, 1, 1)),
    6: ((1, 1, 1),),
    7: ((0, 0, 1),),
}
PRODUCTS = (5, 3, 1, 2, 4, 7, 6)

F32 = jnp.float32
BF16 = jnp.bfloat16


def _strassen_operands(i, a, b):
    def add(u, v):
        return (u.astype(F32) + v.astype(F32)).astype(BF16)

    def sub(u, v):
        return (u.astype(F32) - v.astype(F32)).astype(BF16)

    if i == 1:
        return add(a(0, 0), a(1, 1)), add(b(0, 0), b(1, 1))
    if i == 2:
        return add(a(1, 0), a(1, 1)), b(0, 0)
    if i == 3:
        return a(0, 0), sub(b(0, 1), b(1, 1))
    if i == 4:
        return a(1, 1), sub(b(1, 0), b(0, 0))
    if i == 5:
        return add(a(0, 0), a(0, 1)), b(1, 1)
    if i == 6:
        return sub(a(1, 0), a(0, 0)), add(b(0, 0), b(0, 1))
    return sub(a(0, 1), a(1, 1)), add(b(1, 0), b(1, 1))


def _touches(r, c):
    return [n for n, i in enumerate(PRODUCTS) if any(u[:2] == (r, c) for u in UPDATES[i])]


def _kernel(x_hbm, k_hbm, v_hbm, wq_hbm, wo_hbm, o_hbm,
            x_buf, wq_buf, wo_buf, kv_buf, q_buf, a_buf, acc, stage, o_acc, q_acc,
            x_sem, w_sem, kv_sem, o_sem, *bufs, NB, H, Sq, Sk, D, Dh):
    s_bufs = bufs[:2]
    p_bufs = bufs[2:2 + U]
    r_bufs = bufs[2 + U:2 + 2 * U]
    NG = H // G
    NS = NG * NB
    W = G * Dh
    HK = Sk // 2
    LB = NB.bit_length() - 1
    assert NB == 1 << LB and NB >= 4 and W == 2 * T and D > 2 * T
    qscale = (Dh ** -0.5) * LOG2E

    def rows(i):
        return slice(i * Sq, (i + 1) * Sq)

    def cols(i):
        return slice(i * T, (i + 1) * T)

    def bg(s):
        return s & (NB - 1), s >> LB

    def x_copy(b):
        return pltpu.make_async_copy(x_hbm.at[b], x_buf.at[b], x_sem.at[b])

    def wq_copy(g):
        return pltpu.make_async_copy(
            wq_hbm.at[:, pl.ds(pl.multiple_of(g * W, W), W)], wq_buf.at[g], w_sem.at[0])

    def wo_copy(g):
        return pltpu.make_async_copy(
            wo_hbm.at[pl.ds(pl.multiple_of(g * W, W), W), :], wo_buf.at[g], w_sem.at[1])

    def k_copy(s, slot):
        b, g = bg(s)
        return pltpu.make_async_copy(
            k_hbm.at[pl.ds(2 * b, 2), pl.ds(g * G, G)], kv_buf.at[slot, 0], kv_sem.at[slot])

    def v_copy(s, slot):
        b, g = bg(s)
        return pltpu.make_async_copy(
            v_hbm.at[pl.ds(2 * b, 2), pl.ds(g * G, G)], kv_buf.at[slot, 1], kv_sem.at[slot])

    def kv_wait(slot):
        pltpu.make_async_copy(kv_buf.at[slot], kv_buf.at[slot], kv_sem.at[slot]).wait()

    def o_copy(b):
        return pltpu.make_async_copy(stage.at[b], o_hbm.at[b], o_sem.at[b])

    def q_proj(b, g):
        for r in range(2):
            q_acc[rows(r)] = jnp.dot(x_buf[b, rows(r), 2 * T:], wq_buf[g, 2 * T:, :],
                                     preferred_element_type=F32)
        for n, i in enumerate(PRODUCTS):
            lhs, rhs = _strassen_operands(i, lambda r, c: x_buf[b, rows(r), cols(c)],
                                          lambda r, c: wq_buf[g, cols(r), cols(c)])
            m = jnp.dot(lhs, rhs, preferred_element_type=F32)
            for r, c, sign in UPDATES[i]:
                old = q_acc[rows(r), cols(c)]
                new = old + m if sign > 0 else old - m
                if n == _touches(r, c)[-1]:
                    q_buf[rows(r), cols(c)] = (new * qscale).astype(BF16)
                else:
                    q_acc[rows(r), cols(c)] = new

    def o_proj(b, g, between):
        def update(r, c, m, sign, first, last):
            old = acc[b, rows(r), c]
            if first:
                old = jnp.where(g == 0, 0.0, old)
            new = old + m if sign > 0 else old - m
            acc[b, rows(r), c] = new
            if last:
                stage[b, rows(r), c] = new.astype(stage.dtype)

        for r in range(2):
            c = slice(2 * T, D)
            m = jnp.dot(a_buf[rows(r)], wo_buf[g, :, c], preferred_element_type=F32)
            update(r, c, m, 1, True, True)
            between(r)
        for n, i in enumerate(PRODUCTS):
            lhs, rhs = _strassen_operands(i, lambda r, c: a_buf[rows(r), cols(c)],
                                          lambda r, c: wo_buf[g, cols(r), cols(c)])
            m = jnp.dot(lhs, rhs, preferred_element_type=F32)
            for r, c, sign in UPDATES[i]:
                t = _touches(r, c)
                update(r, cols(c), m, sign, n == t[0], n == t[-1])
            between(2 + n)

    def qk(slot, u, half):
        c = slice(half * HK, (half + 1) * HK)
        r, h = divmod(u, G)
        s_bufs[u % 2][:, c] = lax.dot_general(
            q_buf[rows(r), h * Dh:(h + 1) * Dh], kv_buf[slot, 0, r, h, c, :],
            (((1,), (1,)), ((), ())), preferred_element_type=F32)

    def softmax(u, chunks, i):
        if i >= len(chunks):
            return
        r = slice(sum(chunks[:i]), sum(chunks[:i + 1]))
        s = s_bufs[u % 2][r, :]
        p = jnp.exp2(s - jnp.max(s, axis=-1, keepdims=True))
        l = jnp.sum(p, axis=-1, keepdims=True)
        p_bufs[u][r, :] = p.astype(BF16)
        inv = pl.reciprocal(l, approx=True)
        inv = inv * (2.0 - l * inv)
        r_bufs[u][r, :] = jnp.broadcast_to(inv, (chunks[i], Dh))

    def pv(slot, u, half):
        c = slice(half * HK, (half + 1) * HK)
        r, h = divmod(u, G)
        o = jnp.dot(p_bufs[u][:, c], kv_buf[slot, 1, r, h, c, :], preferred_element_type=F32)
        if half == 0:
            o_acc[...] = o
        else:
            a_buf[rows(r), h * Dh:(h + 1) * Dh] = ((o_acc[...] + o) * r_bufs[u][...]).astype(BF16)

    def compute(s, slot, front, back, after_q=None, after_attn=None):
        if front:
            q_proj(*bg(s))
        if after_q is not None:
            after_q()
        for u in range(U):
            pieces = ("p0", "p1", "q0", "q1") if u == 0 else ("q0", "p0", "p1", "q1")
            for i, (kind, half) in enumerate(pieces):
                if kind == "p" and back:
                    pv(slot, u, int(half))
                if kind == "q" and front:
                    qk(slot, u, int(half))
                if front and u > 0:
                    softmax(u - 1, SM_ROWS, i)
        if after_attn is not None:
            after_attn()
        if back:
            o_proj(*bg(s - 1), (lambda n: softmax(U - 1, SM_ROWS_LAST, n)) if front else (lambda n: None))
        else:
            softmax(U - 1, (Sq,), 0)

    def start_copies(s, slot):
        b, g = bg(s)

        @pl.when(s + 2 <= NS)
        def _():
            k_copy(jnp.minimum(s + 2, NS - 1), slot).start()
            v_copy(s + 1, slot).start()

        @pl.when(s + 2 < NB)
        def _():
            x_copy(s + 2).start()

        @pl.when((b == 2) & (g + 1 < NG))
        def _():
            wq_copy(g + 1).start()
            wo_copy(g + 1).start()

        @pl.when(s - 2 >= NS - NB)
        def _():
            o_copy(s - 2 - (NS - NB)).start()

    def wait_copies(s, next_slot):
        b, g = bg(s)

        @pl.when(s + 1 < NB)
        def _():
            x_copy(s + 1).wait()

        @pl.when((b == NB - 1) & (g + 1 < NG))
        def _():
            wq_copy(g + 1).wait()
            wo_copy(g + 1).wait()

        kv_wait(next_slot)

    x_copy(0).start()
    wq_copy(0).start()
    k_copy(0, 0).start()
    x_copy(0).wait()
    wq_copy(0).wait()
    x_copy(1).start()
    k_copy(1, 1).start()
    v_copy(0, 1).start()
    wo_copy(0).start()
    compute(0, 0, True, False, after_q=lambda: k_copy(0, 0).wait())
    x_copy(2).start()
    k_copy(2, 0).start()
    v_copy(1, 0).start()
    wo_copy(0).wait()
    wait_copies(0, 1)

    def step(s, slot):
        compute(s, slot, True, True, after_attn=lambda: start_copies(s, slot))
        wait_copies(s, 1 - slot)
        return 1 - slot

    lax.fori_loop(1, NS, step, jnp.int32(1))
    o_copy(NB - 2).start()
    compute(NS, NS % 2, False, True)
    o_copy(NB - 1).start()
    for b in range(NB):
        o_copy(b).wait()


@jax.jit
def pallas_standalone__gqa_block_cached__near_ridge_kernel(
    x: jax.Array,
    k_cache: jax.Array,
    v_cache: jax.Array,
    wq: jax.Array,
    wo: jax.Array,
):
    B, Sq, D = x.shape
    _, H, Sk, Dh = k_cache.shape
    assert wq.shape[1] == H * Dh
    NB = B // 2
    NG = H // G
    hbm = pl.BlockSpec(memory_space=pl.ANY)
    out = pl.pallas_call(
        functools.partial(_kernel, NB=NB, H=H, Sq=Sq, Sk=Sk, D=D, Dh=Dh),
        in_specs=[hbm] * 5,
        out_specs=hbm,
        out_shape=jax.ShapeDtypeStruct((NB, 2 * Sq, D), x.dtype),
        scratch_shapes=[
            pltpu.VMEM((NB, 2 * Sq, D), BF16),
            pltpu.VMEM((NG, D, G * Dh), BF16),
            pltpu.VMEM((NG, G * Dh, D), BF16),
            pltpu.VMEM((2, 2, 2, G, Sk, Dh), BF16),
            pltpu.VMEM((2 * Sq, G * Dh), BF16),
            pltpu.VMEM((2 * Sq, G * Dh), BF16),
            pltpu.VMEM((NB, 2 * Sq, D), F32),
            pltpu.VMEM((NB, 2 * Sq, D), x.dtype),
            pltpu.VMEM((Sq, Dh), F32),
            pltpu.VMEM((2 * Sq, G * Dh), F32),
            pltpu.SemaphoreType.DMA((NB,)),
            pltpu.SemaphoreType.DMA((2,)),
            pltpu.SemaphoreType.DMA((2,)),
            pltpu.SemaphoreType.DMA((NB,)),
        ]
        + [pltpu.VMEM((Sq, Sk), F32)] * 2
        + [pltpu.VMEM((Sq, Sk), BF16)] * U
        + [pltpu.VMEM((Sq, Dh), F32)] * U,
        compiler_params=pltpu.CompilerParams(
            vmem_limit_bytes=100 * 1024 * 1024, disable_bounds_checks=True),
    )(x.reshape(NB, 2 * Sq, D), k_cache, v_cache, wq, wo)
    return out.reshape(B, Sq, D)
```
